```python
import jax
import jax.numpy as jnp

def _softmax(x, axis=-1):
    return jax.nn.softmax(x, axis=axis)
def _gelu(x):
    return jax.nn.gelu(x, approximate=True)
def _silu(x):
    return jax.nn.silu(x)
def _sigmoid(x):
    return jax.nn.sigmoid(x)
def _layernorm(x, axis=-1, eps=1e-5):
    m = jnp.mean(x, axis=axis, keepdims=True)
    v = jnp.var(x, axis=axis, keepdims=True)
    return (x - m) / jnp.sqrt(v + eps)
def _scatter_add(tgt, idx, src, axis=0):
    return tgt.at[idx].add(src)
def _segment_sum(src, seg, n):
    return jax.ops.segment_sum(src, seg, n)
class _Rng:
    def __init__(self, key):
        self._k = key
    def _next(self):
        self._k, sub = jax.random.split(self._k)
        return sub
    def normal(self, shape):
        return jax.random.normal(self._next(), shape, dtype=jnp.bfloat16)
    def randint(self, lo, hi, shape):
        return jax.random.randint(self._next(), shape, lo, hi, dtype=jnp.int32)
    def uniform(self, shape, lo=0.0, hi=1.0):
        return jax.random.uniform(self._next(), shape, jnp.bfloat16, lo, hi)
    def permutation(self, n):
        return jax.random.permutation(self._next(), n)


kernel_name = 'sequential_preLN__sliding_block__glu_gated_glu__prompt'

def _fwd_setup_inputs():
    _rng = _Rng(jax.random.key(int.from_bytes(__import__("os").urandom(4), "little")))
    _w = (lambda a: (lambda t: t.astype(jnp.bfloat16) if jnp.issubdtype(t.dtype, jnp.floating) else t)(jnp.asarray(a)))
    def _A_setup():
        B, S, D = 1, 2048, 512
        return {
            "x": _w((lambda *s: _rng.normal(s) * 0.05)(B, S, D)),
            "wqkv": _w((lambda *s: _rng.normal(s) * 0.05)(D, 3 * D)),
            "wo": _w((lambda *s: _rng.normal(s) * 0.05)(D, D)),
        }
    _A_in = _A_setup()

    def _B_setup():
        B, S, D, F = 1, 2048, 512, 1376
        return {
            "x": _w((lambda *s: _rng.normal(s) * 0.05)(B, S, D)),
            "w_gate": _w((lambda *s: _rng.normal(s) * 0.05)(D, F)),
            "w_up": _w((lambda *s: _rng.normal(s) * 0.05)(D, F)),
            "w_down": _w((lambda *s: _rng.normal(s) * 0.05)(F, D)),
        }
    _B_in = _B_setup()

    return {
        "A_x": _A_in["x"],
        "A_wqkv": _A_in["wqkv"],
        "A_wo": _A_in["wo"],
        "B_x": _B_in["x"],
        "B_w_gate": _B_in["w_gate"],
        "B_w_up": _B_in["w_up"],
        "B_w_down": _B_in["w_down"],
    }

def _fwd_reference(A_x, A_wqkv, A_wo, B_x, B_w_gate, B_w_up, B_w_down):
    def _A_ref(x, wqkv, wo):
        B, S, D = x.shape
        H = 32; Dh = D // H; W = 256
        qkv = (lambda x, *d: x.transpose(*d))((x @ wqkv).reshape(B, S, 3, H, Dh), 2, 0, 3, 1, 4)
        q, k, v = qkv[0], qkv[1], qkv[2]
        scores = jnp.einsum("bhqd,bhkd->bhqk", q, k) * (Dh ** -0.5)
        idx = jnp.arange(S)
        mask = (idx[:, None] - idx[None, :] >= 0) & (idx[:, None] - idx[None, :] < W)
        scores = jnp.where(mask[None, None], scores, -1e9)
        p = _softmax(scores, axis=-1)
        o = jnp.einsum("bhqk,bhkd->bhqd", p, v)
        return (lambda x, *d: x.transpose(*d))(o, 0, 2, 1, 3).reshape(B, S, D) @ wo

    def _B_ref(x, w_gate, w_up, w_down):
        g = jnp.einsum("bsd,df->bsf", x, w_gate)
        u = jnp.einsum("bsd,df->bsf", x, w_up)
        h = _sigmoid(g) * u
        return jnp.einsum("bsf,fd->bsd", h, w_down)

    x = A_x
    h = x + _A_ref(_layernorm(x, axis=-1), A_wqkv, A_wo)
    h2 = h + _B_ref(_layernorm(h, axis=-1), B_w_gate, B_w_up, B_w_down)
    return h2


def setup_inputs():
    _inp = _fwd_setup_inputs()
    _gk = jax.random.fold_in(jax.random.key(int.from_bytes(__import__("os").urandom(4), "little")), 2**31 - 1)
    _shapes = [[1, 2048, 512]]
    _dtypes = ['bfloat16']
    _gks = jax.random.split(_gk, len(_shapes))
    _gs = [jax.random.normal(k, s, dtype=jnp.dtype(d)) * 0.05 for k, s, d in zip(_gks, _shapes, _dtypes)]
    _inp["grad_out"] = _gs[0]
    return _inp

def reference(A_x, A_wqkv, A_wo, B_w_gate, B_w_up, B_w_down, B_x, grad_out):
    _const = dict(B_x=B_x)
    def _f(*_d):
        return _fwd_reference(**{'A_x': _d[0], 'A_wqkv': _d[1], 'A_wo': _d[2], 'B_w_gate': _d[3], 'B_w_up': _d[4], 'B_w_down': _d[5], **_const})
    _out, _vjp = jax.vjp(_f, A_x, A_wqkv, A_wo, B_w_gate, B_w_up, B_w_down)
    _grads = _vjp(grad_out)
    _out0 = jnp.asarray(_out)
    return (_out0, *[jnp.asarray(_g) for _g in _grads])
```

```python
import jax
import jax.numpy as jnp
from jax import lax
import jax.experimental.pallas as pl
import jax.experimental.pallas.tpu as pltpu

S = 2048
D = 512
F = 1376
H = 32
DH = 16
W = 256
NG = 4
T = 256
BQ = 128
WIN = W + BQ
NL = 8 * BQ
NT_ = S // T
NSB = T // BQ
EPS = 1e-5
NEG = -1e9
LOG2E = 1.4426950408889634
QSCALE = DH ** -0.5 * LOG2E
BF = jnp.bfloat16
F32 = jnp.float32

_NN = (((1,), (0,)), ((), ()))
_NT = (((1,), (1,)), ((), ()))
_TN = (((0,), (0,)), ((), ()))
_TT = (((0,), (1,)), ((), ()))


def _dot(a, b, dims):
    return lax.dot_general(a, b, dims, preferred_element_type=F32)


def _ln(x):
    m = jnp.mean(x, axis=-1, keepdims=True)
    xc = x - m
    v = jnp.mean(xc * xc, axis=-1, keepdims=True)
    rstd = lax.rsqrt(v + EPS)
    return xc * rstd, rstd


def _ln_bwd(dy, y, rstd):
    m1 = jnp.mean(dy, axis=-1, keepdims=True)
    m2 = jnp.mean(dy * y, axis=-1, keepdims=True)
    return rstd * (dy - m1 - y * m2)


def _kernel(x_ref, dout_ref, wqkv_hbm, wo_hbm, wg_hbm, wu_hbm, wd_hbm,
            out_ref, dx_ref, dwqkv_hbm, dwo_hbm, dwg_hbm, dwu_hbm, dwd_hbm,
            wqkv_ref, wo_ref, wg_ref, wu_ref, wd_ref, in_sem, out_sem,
            k_buf, v_buf, kt_buf, vt_buf, dkt_buf, dvt_buf, qt_buf, p_buf, linv_buf,
            ot_buf, dot_buf, dqt_buf, dh_buf, n1_buf, rs_buf,
            a_qkv, a_o, a_g, a_u, a_d):
    i = pl.program_id(0)
    slot = i % 2

    def in_copy(k):
        src = (wqkv_hbm, wo_hbm, wg_hbm, wu_hbm, wd_hbm)[k]
        dst = (wqkv_ref, wo_ref, wg_ref, wu_ref, wd_ref)[k]
        return pltpu.make_async_copy(src, dst, in_sem.at[k])

    def out_copy(k):
        src = (wqkv_ref, wo_ref, wg_ref, wu_ref, wd_ref)[k]
        dst = (dwqkv_hbm, dwo_hbm, dwg_hbm, dwu_hbm, dwd_hbm)[k]
        return pltpu.make_async_copy(src, dst, out_sem.at[k])

    @pl.when(i == 0)
    def _init():
        for k in range(5):
            in_copy(k).start()
        k_buf[:, 0:W, :] = jnp.zeros((NG, W, 128), BF)
        v_buf[:, 0:W, :] = jnp.zeros((NG, W, 128), BF)
        kt_buf[:, :, 0:W] = jnp.zeros((NG, 128, W), BF)
        vt_buf[:, :, 0:W] = jnp.zeros((NG, 128, W), BF)
        dkt_buf[...] = jnp.zeros_like(dkt_buf)
        dvt_buf[...] = jnp.zeros_like(dvt_buf)
        in_copy(0).wait()

    def acc(ref, first):
        return jnp.where(first, 0.0, ref[...])

    row_h = lax.broadcasted_iota(jnp.int32, (128, NL), 0) // DH
    lane_h = lax.broadcasted_iota(jnp.int32, (128, NL), 1) // BQ
    hmask_t = row_h == lane_h

    def stack_t(a):
        return jnp.where(hmask_t, jnp.concatenate([a] * 8, axis=1), 0.0)

    @pl.when(i < NT_)
    def _main():
        row0 = pl.multiple_of(i * T, T)
        x = x_ref[...].astype(F32)
        n1, rstd1 = _ln(x)
        n1b = n1.astype(BF)
        n1_buf[slot] = n1b
        rs_buf[slot] = jnp.broadcast_to(rstd1, (T, 128))
        qkv = _dot(n1b, wqkv_ref[...], _NN)
        qt_buf[...] = (qkv[:, 0:D] * QSCALE).T.reshape(NG, 128, T)
        kt = qkv[:, D:2 * D].T.astype(BF)
        vt = qkv[:, 2 * D:3 * D].T.astype(BF)
        for g in range(NG):
            k_buf[g, pl.ds(W + row0, T), :] = qkv[:, D + g * 128:D + (g + 1) * 128].astype(BF)
            v_buf[g, pl.ds(W + row0, T), :] = qkv[:, 2 * D + g * 128:2 * D + (g + 1) * 128].astype(BF)
            kt_buf[g, :, pl.ds(W + row0, T)] = kt[g * 128:(g + 1) * 128, :]
            vt_buf[g, :, pl.ds(W + row0, T)] = vt[g * 128:(g + 1) * 128, :]

        kk = lax.broadcasted_iota(jnp.int32, (BQ, BQ), 0)
        qq = lax.broadcasted_iota(jnp.int32, (BQ, BQ), 1)
        bias_lo = jnp.where(kk > qq, 0.0, NEG)
        bias_hi = jnp.where(kk <= qq, 0.0, NEG)

        def tile8(b):
            return jnp.concatenate([b] * 8, axis=1)

        def fwd_body(j, carry):
            r0 = pl.multiple_of(j * BQ, BQ)
            start = pl.multiple_of(row0 + r0, BQ)
            lim = W - start
            b0 = jnp.where(kk >= lim, bias_lo, NEG)
            b1 = jnp.where(kk >= lim - BQ, 0.0, NEG)

            def scores(g):
                kw = k_buf[g, pl.ds(start, WIN), :]
                qm = stack_t(qt_buf[g, :, pl.ds(r0, BQ)]).astype(BF)
                return _dot(kw, qm, _NN)

            def softmax(g, s):
                s0 = s[0:BQ] + tile8(b0)
                s1 = s[BQ:2 * BQ] + tile8(b1)
                s2 = s[2 * BQ:3 * BQ] + tile8(bias_hi)
                m = jnp.max(jnp.maximum(jnp.maximum(s0, s1), s2), axis=0, keepdims=True)
                p0 = jnp.exp2(s0 - m)
                p1 = jnp.exp2(s1 - m)
                p2 = jnp.exp2(s2 - m)
                l = jnp.sum(p0 + p1 + p2, axis=0, keepdims=True)
                linv = 1.0 / l
                pb = jnp.concatenate([p0.astype(BF), p1.astype(BF), p2.astype(BF)], axis=0)
                p_buf[j, g] = pb
                linv_buf[j, g] = jnp.broadcast_to(linv, (8, NL))

            def pv(g):
                vtw = vt_buf[g, :, pl.ds(start, WIN)]
                pb = p_buf[j, g]
                linv = linv_buf[j, g][0:1, :]
                ot_buf[g * 128:(g + 1) * 128, pl.ds(r0, BQ)] = jnp.concatenate([
                    _dot(vtw[h * DH:(h + 1) * DH, :], pb[:, h * BQ:(h + 1) * BQ], _NN)
                    * linv[:, h * BQ:(h + 1) * BQ] for h in range(8)], axis=0)

            s_next = scores(0)
            for g in range(NG):
                s = s_next
                if g + 1 < NG:
                    s_next = scores(g + 1)
                if g > 0:
                    pv(g - 1)
                softmax(g, s)
            pv(NG - 1)
            return carry

        lax.fori_loop(0, NSB, fwd_body, 0)

        @pl.when(i == 0)
        def _():
            for k in range(1, 5):
                in_copy(k).wait()

        otb = ot_buf[...].astype(BF)
        h = x + _dot(otb, wo_ref[...], _TN)
        n2, rstd2 = _ln(h)
        n2b = n2.astype(BF)
        gt = _dot(n2b, wg_ref[...], _NT)
        ut = _dot(n2b, wu_ref[...], _NT)
        sg = jax.nn.sigmoid(gt)
        hh = (sg * ut).astype(BF)
        h2 = h + _dot(hh, wd_ref[...], _NN)
        out_ref[...] = h2.astype(out_ref.dtype)

        dout = dout_ref[...]
        dhh = _dot(dout, wd_ref[...], _NT)
        a_d[...] = acc(a_d, i == 0) + _dot(hh, dout, _TN)
        du = (dhh * sg).astype(BF)
        dg = (dhh * ut * sg * (1.0 - sg)).astype(BF)
        a_g[...] = acc(a_g, i == 0) + _dot(dg, n2b, _TN)
        a_u[...] = acc(a_u, i == 0) + _dot(du, n2b, _TN)
        dn2 = _dot(dg, wg_ref[...], _NN) + _dot(du, wu_ref[...], _NN)
        dh = dout.astype(F32) + _ln_bwd(dn2, n2, rstd2)
        dh_buf[slot] = dh
        dhb = dh.astype(BF)
        a_o[...] = acc(a_o, i == 0) + _dot(otb, dhb, _NN)
        dot_buf[...] = _dot(wo_ref[...], dhb, _NT)

        def bwd_body(j, carry):
            r0 = pl.multiple_of(j * BQ, BQ)
            start = pl.multiple_of(row0 + r0, BQ)
            for g in range(NG):
                vw = v_buf[g, pl.ds(start, WIN), :]
                ktw = kt_buf[g, :, pl.ds(start, WIN)]
                dot_g = dot_buf[g * 128:(g + 1) * 128, pl.ds(r0, BQ)]
                qt = qt_buf[g, :, pl.ds(r0, BQ)].astype(BF)
                linv = linv_buf[j, g][0:1, :]
                pb = p_buf[j, g]
                p = pb.astype(F32)
                dom = (stack_t(dot_g) * linv).astype(BF)
                prod = dot_g * ot_buf[g * 128:(g + 1) * 128, pl.ds(r0, BQ)]
                dl = jnp.sum(prod.reshape(8, DH, BQ), axis=1)
                delta = jnp.concatenate([dl[h:h + 1, :] for h in range(8)], axis=1) * linv
                dp = _dot(vw, dom, _NN)
                dsf = p * (dp - delta)
                ds = dsf.astype(BF)
                dsq = dsf.T.astype(BF)
                dvs, dks, dqs = [], [], []
                for h in range(8):
                    rows = slice(h * DH, (h + 1) * DH)
                    cols = slice(h * BQ, (h + 1) * BQ)
                    dvs.append(_dot(dom[rows, cols], pb[:, cols], _NT))
                    dks.append(_dot(qt[rows, :], dsq[cols, :], _NN))
                    dqs.append(_dot(ktw[rows, :], ds[:, cols], _NN))
                dvt_buf[g, :, pl.ds(start, WIN)] += jnp.concatenate(dvs, axis=0)
                dkt_buf[g, :, pl.ds(start, WIN)] += jnp.concatenate(dks, axis=0)
                dqt_buf[slot, g * 128:(g + 1) * 128, pl.ds(r0, BQ)] = jnp.concatenate(dqs, axis=0)
            return carry

        lax.fori_loop(0, NSB, bwd_body, 0, unroll=True)

    @pl.when(i == NT_)
    def _write_early():
        wo_ref[...] = a_o[...].astype(BF)
        wg_ref[...] = a_g[...].astype(BF)
        wu_ref[...] = a_u[...].astype(BF)
        wd_ref[...] = a_d[...].astype(BF)
        for k in range(1, 5):
            out_copy(k).start()

    @pl.when(i > 0)
    def _final():
        ps = 1 - slot
        prow = pl.multiple_of(W + (i - 1) * T, T)
        n1b = n1_buf[ps]
        n1 = n1b.astype(F32)
        rstd1 = rs_buf[ps][:, 0:1]
        parts = [(dqt_buf[ps] * (DH ** -0.5)).astype(BF)]
        parts += [(dkt_buf[g, :, pl.ds(prow, T)] * (1.0 / LOG2E)).astype(BF) for g in range(NG)]
        parts += [dvt_buf[g, :, pl.ds(prow, T)].astype(BF) for g in range(NG)]
        dqkvt = jnp.concatenate(parts, axis=0)
        a_qkv[...] = acc(a_qkv, i == 1) + _dot(dqkvt, n1b, _NN)
        dn1 = _dot(dqkvt, wqkv_ref[...], _TT)
        dx = dh_buf[ps] + _ln_bwd(dn1, n1, rstd1)
        dx_ref[...] = dx.astype(dx_ref.dtype)

    @pl.when(i == NT_)
    def _write():
        wqkv_ref[...] = a_qkv[...].T.astype(BF)
        out_copy(0).start()
        for k in range(5):
            out_copy(k).wait()


@jax.jit
def pallas_sequential_preLN__sliding_block__glu_gated_glu__prompt_kernel(
    A_x, A_wqkv, A_wo, B_x, B_w_gate, B_w_up, B_w_down, grad_out):
    x = A_x.reshape(S, D)
    dout = grad_out.reshape(S, D)

    cur = lambda i: (jnp.minimum(i, NT_ - 1), 0)
    prev = lambda i: (jnp.maximum(i - 1, 0), 0)
    hbm = pl.BlockSpec(memory_space=pl.ANY)

    outs = pl.pallas_call(
        _kernel,
        grid=(NT_ + 1,),
        in_specs=[
            pl.BlockSpec((T, D), cur),
            pl.BlockSpec((T, D), cur),
            hbm, hbm, hbm, hbm, hbm,
        ],
        out_specs=[
            pl.BlockSpec((T, D), cur),
            pl.BlockSpec((T, D), prev),
            hbm, hbm, hbm, hbm, hbm,
        ],
        out_shape=[
            jax.ShapeDtypeStruct((S, D), BF),
            jax.ShapeDtypeStruct((S, D), BF),
            jax.ShapeDtypeStruct((D, 3 * D), BF),
            jax.ShapeDtypeStruct((D, D), BF),
            jax.ShapeDtypeStruct((F, D), BF),
            jax.ShapeDtypeStruct((F, D), BF),
            jax.ShapeDtypeStruct((F, D), BF),
        ],
        scratch_shapes=[
            pltpu.VMEM((D, 3 * D), BF),
            pltpu.VMEM((D, D), BF),
            pltpu.VMEM((F, D), BF),
            pltpu.VMEM((F, D), BF),
            pltpu.VMEM((F, D), BF),
            pltpu.SemaphoreType.DMA((5,)),
            pltpu.SemaphoreType.DMA((5,)),
            pltpu.VMEM((NG, W + S, 128), BF),
            pltpu.VMEM((NG, W + S, 128), BF),
            pltpu.VMEM((NG, 128, W + S), BF),
            pltpu.VMEM((NG, 128, W + S), BF),
            pltpu.VMEM((NG, 128, W + S), F32),
            pltpu.VMEM((NG, 128, W + S), F32),
            pltpu.VMEM((NG, 128, T), F32),
            pltpu.VMEM((NSB, NG, WIN, NL), BF),
            pltpu.VMEM((NSB, NG, 8, NL), F32),
            pltpu.VMEM((D, T), F32),
            pltpu.VMEM((D, T), F32),
            pltpu.VMEM((2, D, T), F32),
            pltpu.VMEM((2, T, D), F32),
            pltpu.VMEM((2, T, D), BF),
            pltpu.VMEM((2, T, 128), F32),
            pltpu.VMEM((3 * D, D), F32),
            pltpu.VMEM((D, D), F32),
            pltpu.VMEM((F, D), F32),
            pltpu.VMEM((F, D), F32),
            pltpu.VMEM((F, D), F32),
        ],
        compiler_params=pltpu.CompilerParams(
            dimension_semantics=("arbitrary",),
            vmem_limit_bytes=100 * 1024 * 1024,
        ),
    )(x, dout, A_wqkv, A_wo, B_w_gate.T, B_w_up.T, B_w_down)
    h2, dx, dwqkv, dwo, dwg, dwu, dwd = outs
    return (h2.reshape(1, S, D), dx.reshape(1, S, D), dwqkv, dwo, dwg.T, dwu.T, dwd)
```

```python
import jax
import jax.numpy as jnp
from jax import lax
import jax.experimental.pallas as pl
import jax.experimental.pallas.tpu as pltpu

S = 2048
D = 512
F = 1376
DH = 16
W = 256
NG = 4
T = 256
BQ = 128
WIN = W + BQ
NL = 8 * BQ
NT_ = S // T
NSB = T // BQ
EPS = 1e-5
NEG = -1e9
LOG2E = 1.4426950408889634
QSCALE = DH ** -0.5 * LOG2E
BF = jnp.bfloat16
F32 = jnp.float32

_NN = (((1,), (0,)), ((), ()))
_NT = (((1,), (1,)), ((), ()))
_TN = (((0,), (0,)), ((), ()))
_TT = (((0,), (1,)), ((), ()))


def _dot(a, b, dims):
    return lax.dot_general(a, b, dims, preferred_element_type=F32)


def _ln(x):
    m = jnp.mean(x, axis=-1, keepdims=True)
    xc = x - m
    v = jnp.mean(xc * xc, axis=-1, keepdims=True)
    rstd = lax.rsqrt(v + EPS)
    return xc * rstd, rstd


def _ln_bwd(dy, y, rstd):
    m1 = jnp.mean(dy, axis=-1, keepdims=True)
    m2 = jnp.mean(dy * y, axis=-1, keepdims=True)
    return rstd * (dy - m1 - y * m2)


def _kernel(x_ref, dout_ref, wqkv_hbm, wo_hbm, wg_hbm, wu_hbm, wd_hbm,
            out_ref, dx_ref, dwqkv_hbm, dwo_hbm, dwg_hbm, dwu_hbm, dwd_hbm,
            wqkv_ref, wo_ref, wg_ref, wu_ref, wd_ref, in_sem, out_sem,
            k_buf, v_buf, kt_buf, vt_buf, dkt_buf, dvt_buf, qt_buf, p_buf, linv_buf,
            ot_buf, dot_buf, dqt_buf, dh_buf, n1_buf, rs_buf,
            a_qkv, a_o, a_g, a_u, a_d):
    i = pl.program_id(0)
    slot = i % 2

    def in_copy(k):
        src = (wqkv_hbm, wo_hbm, wg_hbm, wu_hbm, wd_hbm)[k]
        dst = (wqkv_ref, wo_ref, wg_ref, wu_ref, wd_ref)[k]
        return pltpu.make_async_copy(src, dst, in_sem.at[k])

    def out_copy(k):
        src = (wqkv_ref, wo_ref, wg_ref, wu_ref, wd_ref)[k]
        dst = (dwqkv_hbm, dwo_hbm, dwg_hbm, dwu_hbm, dwd_hbm)[k]
        return pltpu.make_async_copy(src, dst, out_sem.at[k])

    @pl.when(i == 0)
    def _init():
        for k in range(5):
            in_copy(k).start()
        k_buf[:, 0:W, :] = jnp.zeros((NG, W, 128), BF)
        v_buf[:, 0:W, :] = jnp.zeros((NG, W, 128), BF)
        kt_buf[:, :, 0:W] = jnp.zeros((NG, 128, W), BF)
        vt_buf[:, :, 0:W] = jnp.zeros((NG, 128, W), BF)
        dkt_buf[...] = jnp.zeros_like(dkt_buf)
        dvt_buf[...] = jnp.zeros_like(dvt_buf)
        in_copy(0).wait()

    def acc(ref, first):
        return jnp.where(first, 0.0, ref[...])

    row_h = lax.broadcasted_iota(jnp.int32, (128, NL), 0) // DH
    lane_h = lax.broadcasted_iota(jnp.int32, (128, NL), 1) // BQ
    hmask_t = row_h == lane_h

    def stack_t(a):
        return jnp.where(hmask_t, jnp.concatenate([a] * 8, axis=1), 0.0)

    @pl.when(i < NT_)
    def _main():
        row0 = pl.multiple_of(i * T, T)
        x = x_ref[...].astype(F32)
        n1, rstd1 = _ln(x)
        n1b = n1.astype(BF)
        n1_buf[slot] = n1b
        rs_buf[slot] = jnp.broadcast_to(rstd1, (T, 128))
        qkv = _dot(n1b, wqkv_ref[...], _NN)
        qt_buf[...] = (qkv[:, 0:D] * QSCALE).T.reshape(NG, 128, T)
        kt = qkv[:, D:2 * D].T.astype(BF)
        vt = qkv[:, 2 * D:3 * D].T.astype(BF)
        for g in range(NG):
            k_buf[g, pl.ds(W + row0, T), :] = qkv[:, D + g * 128:D + (g + 1) * 128].astype(BF)
            v_buf[g, pl.ds(W + row0, T), :] = qkv[:, 2 * D + g * 128:2 * D + (g + 1) * 128].astype(BF)
            kt_buf[g, :, pl.ds(W + row0, T)] = kt[g * 128:(g + 1) * 128, :]
            vt_buf[g, :, pl.ds(W + row0, T)] = vt[g * 128:(g + 1) * 128, :]

        kk = lax.broadcasted_iota(jnp.int32, (BQ, BQ), 0)
        qq = lax.broadcasted_iota(jnp.int32, (BQ, BQ), 1)
        bias_lo = jnp.where(kk > qq, 0.0, NEG)
        bias_hi = jnp.where(kk <= qq, 0.0, NEG)

        def tile8(b):
            return jnp.concatenate([b] * 8, axis=1)

        def fwd_body(j, carry):
            r0 = pl.multiple_of(j * BQ, BQ)
            start = pl.multiple_of(row0 + r0, BQ)
            lim = W - start
            b0 = jnp.where(kk >= lim, bias_lo, NEG)
            b1 = jnp.where(kk >= lim - BQ, 0.0, NEG)

            def scores(g):
                kw = k_buf[g, pl.ds(start, WIN), :]
                qm = stack_t(qt_buf[g, :, pl.ds(r0, BQ)]).astype(BF)
                return _dot(kw, qm, _NN)

            def softmax(g, s):
                ps, ms, ls = [], [], []
                for c, b in enumerate((b0, b1, bias_hi)):
                    sc = s[c * BQ:(c + 1) * BQ] + tile8(b)
                    mc = jnp.max(sc, axis=0, keepdims=True)
                    pc = jnp.exp2(sc - mc)
                    ls.append(jnp.sum(pc, axis=0, keepdims=True))
                    ms.append(mc)
                    ps.append(pc.astype(BF))
                m = jnp.maximum(jnp.maximum(ms[0], ms[1]), ms[2])
                cs = [jnp.exp2(mc - m) for mc in ms]
                linv = 1.0 / (cs[0] * ls[0] + cs[1] * ls[1] + cs[2] * ls[2])
                p_buf[j, g] = jnp.concatenate(ps, axis=0)
                linv_buf[j, g] = jnp.concatenate(
                    [c_ * linv for c_ in cs] + cs + [linv, linv], axis=0)

            def pv(g):
                vtw = vt_buf[g, :, pl.ds(start, WIN)]
                pb = p_buf[j, g]
                wts = linv_buf[j, g]
                outs = []
                for h in range(8):
                    rows = slice(h * DH, (h + 1) * DH)
                    cols = slice(h * BQ, (h + 1) * BQ)
                    o = None
                    for c in range(3):
                        kc = slice(c * BQ, (c + 1) * BQ)
                        t_ = _dot(vtw[rows, kc], pb[kc, cols], _NN) * wts[c:c + 1, cols]
                        o = t_ if o is None else o + t_
                    outs.append(o)
                ot_buf[g * 128:(g + 1) * 128, pl.ds(r0, BQ)] = jnp.concatenate(outs, axis=0)

            s_next = scores(0)
            for g in range(NG):
                s = s_next
                if g + 1 < NG:
                    s_next = scores(g + 1)
                if g > 0:
                    pv(g - 1)
                softmax(g, s)
            pv(NG - 1)
            return carry

        lax.fori_loop(0, NSB, fwd_body, 0)

        @pl.when(i == 0)
        def _():
            for k in range(1, 5):
                in_copy(k).wait()

        otb = ot_buf[...].astype(BF)
        h = x + _dot(otb, wo_ref[...], _TN)
        n2, rstd2 = _ln(h)
        n2b = n2.astype(BF)
        gt = _dot(n2b, wg_ref[...], _NT)
        ut = _dot(n2b, wu_ref[...], _NT)
        sg = jax.nn.sigmoid(gt)
        hh = (sg * ut).astype(BF)
        h2 = h + _dot(hh, wd_ref[...], _NN)
        out_ref[...] = h2.astype(out_ref.dtype)

        dout = dout_ref[...]
        dhh = _dot(dout, wd_ref[...], _NT)
        a_d[...] = acc(a_d, i == 0) + _dot(hh, dout, _TN)
        du = (dhh * sg).astype(BF)
        dg = (dhh * ut * sg * (1.0 - sg)).astype(BF)
        a_g[...] = acc(a_g, i == 0) + _dot(dg, n2b, _TN)
        a_u[...] = acc(a_u, i == 0) + _dot(du, n2b, _TN)
        dn2 = _dot(dg, wg_ref[...], _NN) + _dot(du, wu_ref[...], _NN)
        dh = dout.astype(F32) + _ln_bwd(dn2, n2, rstd2)
        dh_buf[slot] = dh
        dhb = dh.astype(BF)
        a_o[...] = acc(a_o, i == 0) + _dot(otb, dhb, _NN)
        dot_buf[...] = _dot(wo_ref[...], dhb, _NT)

        def bwd_body(j, carry):
            r0 = pl.multiple_of(j * BQ, BQ)
            start = pl.multiple_of(row0 + r0, BQ)
            for g in range(NG):
                vw = v_buf[g, pl.ds(start, WIN), :]
                ktw = kt_buf[g, :, pl.ds(start, WIN)]
                dot_g = dot_buf[g * 128:(g + 1) * 128, pl.ds(r0, BQ)]
                qt = qt_buf[g, :, pl.ds(r0, BQ)].astype(BF)
                wts = linv_buf[j, g]
                linv = wts[6:7, :]
                pb = p_buf[j, g]
                dom = (stack_t(dot_g) * linv).astype(BF)
                prod = dot_g * ot_buf[g * 128:(g + 1) * 128, pl.ds(r0, BQ)]
                dl = jnp.sum(prod.reshape(8, DH, BQ), axis=1)
                delta = jnp.concatenate([dl[h:h + 1, :] for h in range(8)], axis=1) * linv
                dp = _dot(vw, dom, _NN) - delta
                dsf = jnp.concatenate(
                    [pb[c * BQ:(c + 1) * BQ, :].astype(F32) * wts[3 + c:4 + c, :] * dp[c * BQ:(c + 1) * BQ, :]
                     for c in range(3)], axis=0)
                ds = dsf.astype(BF)
                dsq = dsf.T.astype(BF)
                dvs, dks, dqs = [], [], []
                for h in range(8):
                    rows = slice(h * DH, (h + 1) * DH)
                    cols = slice(h * BQ, (h + 1) * BQ)
                    dvs.append(jnp.concatenate(
                        [_dot((dot_g[rows, :] * wts[c:c + 1, cols]).astype(BF), pb[c * BQ:(c + 1) * BQ, cols], _NT)
                         for c in range(3)], axis=1))
                    dks.append(_dot(qt[rows, :], dsq[cols, :], _NN))
                    dqs.append(_dot(ktw[rows, :], ds[:, cols], _NN))
                dvt_buf[g, :, pl.ds(start, WIN)] += jnp.concatenate(dvs, axis=0)
                dkt_buf[g, :, pl.ds(start, WIN)] += jnp.concatenate(dks, axis=0)
                dqt_buf[slot, g * 128:(g + 1) * 128, pl.ds(r0, BQ)] = jnp.concatenate(dqs, axis=0)
            return carry

        lax.fori_loop(0, NSB, bwd_body, 0)

    @pl.when(i == NT_)
    def _write_early():
        wo_ref[...] = a_o[...].astype(BF)
        wg_ref[...] = a_g[...].astype(BF)
        wu_ref[...] = a_u[...].astype(BF)
        wd_ref[...] = a_d[...].astype(BF)
        for k in range(1, 5):
            out_copy(k).start()

    @pl.when(i > 0)
    def _final():
        ps = 1 - slot
        prow = pl.multiple_of(W + (i - 1) * T, T)
        n1b = n1_buf[ps]
        n1 = n1b.astype(F32)
        rstd1 = rs_buf[ps][:, 0:1]
        parts = [(dqt_buf[ps] * (DH ** -0.5)).astype(BF)]
        parts += [(dkt_buf[g, :, pl.ds(prow, T)] * (1.0 / LOG2E)).astype(BF) for g in range(NG)]
        parts += [dvt_buf[g, :, pl.ds(prow, T)].astype(BF) for g in range(NG)]
        dqkvt = jnp.concatenate(parts, axis=0)
        a_qkv[...] = acc(a_qkv, i == 1) + _dot(dqkvt, n1b, _NN)
        dn1 = _dot(dqkvt, wqkv_ref[...], _TT)
        dx = dh_buf[ps] + _ln_bwd(dn1, n1, rstd1)
        dx_ref[...] = dx.astype(dx_ref.dtype)

    @pl.when(i == NT_)
    def _write():
        wqkv_ref[...] = a_qkv[...].T.astype(BF)
        out_copy(0).start()
        for k in range(5):
            out_copy(k).wait()


@jax.jit
def pallas_sequential_preLN__sliding_block__glu_gated_glu__prompt_kernel(
    A_x, A_wqkv, A_wo, B_x, B_w_gate, B_w_up, B_w_down, grad_out):
    x = A_x.reshape(S, D)
    dout = grad_out.reshape(S, D)

    cur = lambda i: (jnp.minimum(i, NT_ - 1), 0)
    prev = lambda i: (jnp.maximum(i - 1, 0), 0)
    hbm = pl.BlockSpec(memory_space=pl.ANY)

    outs = pl.pallas_call(
        _kernel,
        grid=(NT_ + 1,),
        in_specs=[
            pl.BlockSpec((T, D), cur),
            pl.BlockSpec((T, D), cur),
            hbm, hbm, hbm, hbm, hbm,
        ],
        out_specs=[
            pl.BlockSpec((T, D), cur),
            pl.BlockSpec((T, D), prev),
            hbm, hbm, hbm, hbm, hbm,
        ],
        out_shape=[
            jax.ShapeDtypeStruct((S, D), BF),
            jax.ShapeDtypeStruct((S, D), BF),
            jax.ShapeDtypeStruct((D, 3 * D), BF),
            jax.ShapeDtypeStruct((D, D), BF),
            jax.ShapeDtypeStruct((F, D), BF),
            jax.ShapeDtypeStruct((F, D), BF),
            jax.ShapeDtypeStruct((F, D), BF),
        ],
        scratch_shapes=[
            pltpu.VMEM((D, 3 * D), BF),
            pltpu.VMEM((D, D), BF),
            pltpu.VMEM((F, D), BF),
            pltpu.VMEM((F, D), BF),
            pltpu.VMEM((F, D), BF),
            pltpu.SemaphoreType.DMA((5,)),
            pltpu.SemaphoreType.DMA((5,)),
            pltpu.VMEM((NG, W + S, 128), BF),
            pltpu.VMEM((NG, W + S, 128), BF),
            pltpu.VMEM((NG, 128, W + S), BF),
            pltpu.VMEM((NG, 128, W + S), BF),
            pltpu.VMEM((NG, 128, W + S), F32),
            pltpu.VMEM((NG, 128, W + S), F32),
            pltpu.VMEM((NG, 128, T), F32),
            pltpu.VMEM((NSB, NG, WIN, NL), BF),
            pltpu.VMEM((NSB, NG, 8, NL), F32),
            pltpu.VMEM((D, T), F32),
            pltpu.VMEM((D, T), F32),
            pltpu.VMEM((2, D, T), F32),
            pltpu.VMEM((2, T, D), F32),
            pltpu.VMEM((2, T, D), BF),
            pltpu.VMEM((2, T, 128), F32),
            pltpu.VMEM((3 * D, D), F32),
            pltpu.VMEM((D, D), F32),
            pltpu.VMEM((F, D), F32),
            pltpu.VMEM((F, D), F32),
            pltpu.VMEM((F, D), F32),
        ],
        compiler_params=pltpu.CompilerParams(
            dimension_semantics=("arbitrary",),
            vmem_limit_bytes=100 * 1024 * 1024,
        ),
    )(x, dout, A_wqkv, A_wo, B_w_gate.T, B_w_up.T, B_w_down)
    h2, dx, dwqkv, dwo, dwg, dwu, dwd = outs
    return (h2.reshape(1, S, D), dx.reshape(1, S, D), dwqkv, dwo, dwg.T, dwu.T, dwd)
```
